```python
import os as _os
_os.environ.setdefault("JAX_PLATFORMS", "cpu")
import jax
import jax.numpy as jnp

def _softmax(x, axis=-1):
    return jax.nn.softmax(x, axis=axis)
def _gelu(x):
    return jax.nn.gelu(x, approximate=True)
def _silu(x):
    return jax.nn.silu(x)
def _sigmoid(x):
    return jax.nn.sigmoid(x)
def _layernorm(x, axis=-1, eps=1e-5):
    m = jnp.mean(x, axis=axis, keepdims=True)
    v = jnp.var(x, axis=axis, keepdims=True)
    return (x - m) / jnp.sqrt(v + eps)
def _scatter_add(tgt, idx, src, axis=0):
    return tgt.at[idx].add(src)
def _segment_sum(src, seg, n):
    return jax.ops.segment_sum(src, seg, n)
class _Rng:
    def __init__(self, key):
        self._k = key
    def _next(self):
        self._k, sub = jax.random.split(self._k)
        return sub
    def normal(self, shape):
        return jax.random.normal(self._next(), shape, dtype=jnp.bfloat16)
    def randint(self, lo, hi, shape):
        return jax.random.randint(self._next(), shape, lo, hi, dtype=jnp.int32)
    def uniform(self, shape, lo=0.0, hi=1.0):
        return jax.random.uniform(self._next(), shape, jnp.bfloat16, lo, hi)
    def permutation(self, n):
        return jax.random.permutation(self._next(), n)


kernel_name = 'gated_mix__ssm_conv_s5__glu_gated_geglu__prompt'

def setup_inputs():
    _rng = _Rng(jax.random.key(int.from_bytes(__import__("os").urandom(4), "little")))
    _w = (lambda a: (lambda t: t.astype(jnp.bfloat16) if jnp.issubdtype(t.dtype, jnp.floating) else t)(jnp.asarray(a)))
    def _A_setup():
        B, S, D = 1, 2048, 448
        P = D
        Lambda_re = -0.5 * jnp.exp((lambda *s: _rng.normal(s) * 0.4)(P))
        Lambda_im = (lambda *s: _rng.normal(s) * 0.4)(P) * 1.0
        B_re = (lambda *s: _rng.normal(s) * 0.4)(P, D) * (D ** -0.5)
        B_im = (lambda *s: _rng.normal(s) * 0.4)(P, D) * (D ** -0.5)
        C_re = (lambda *s: _rng.normal(s) * 0.4)(D, P) * (P ** -0.5)
        C_im = (lambda *s: _rng.normal(s) * 0.4)(D, P) * (P ** -0.5)
        log_dt = (lambda *s: _rng.normal(s) * 0.4)(P) * 0.3 - 2.0
        Dskip = (lambda *s: _rng.normal(s) * 0.4)(D)
        return {
            "x": _w((lambda *s: _rng.normal(s) * 0.05)(B, S, D)),
            "Lambda_re": _w(Lambda_re),
            "Lambda_im": _w(Lambda_im),
            "B_re": _w(B_re),
            "B_im": _w(B_im),
            "C_re": _w(C_re),
            "C_im": _w(C_im),
            "log_dt": _w(log_dt),
            "Dskip": _w(Dskip),
        }
    _A_in = _A_setup()

    def _B_setup():
        B, S, Dm, Df = 1, 2048, 448, 1792
        return {
            "x": _w((lambda *s: _rng.normal(s) * 0.05)(B, S, Dm)),
            "w_gate": _w((lambda *s: _rng.normal(s) * 1.6)(Dm, Df) * (Dm ** -0.5)),
            "w_up": _w((lambda *s: _rng.normal(s) * 1.6)(Dm, Df) * (Dm ** -0.5)),
            "w_down": _w((lambda *s: _rng.normal(s) * 1.6)(Df, Dm) * (Df ** -0.5)),
        }
    _B_in = _B_setup()

    return {
        "A_x": _A_in["x"],
        "A_Lambda_re": _A_in["Lambda_re"],
        "A_Lambda_im": _A_in["Lambda_im"],
        "A_B_re": _A_in["B_re"],
        "A_B_im": _A_in["B_im"],
        "A_C_re": _A_in["C_re"],
        "A_C_im": _A_in["C_im"],
        "A_log_dt": _A_in["log_dt"],
        "A_Dskip": _A_in["Dskip"],
        "B_x": _B_in["x"],
        "B_w_gate": _B_in["w_gate"],
        "B_w_up": _B_in["w_up"],
        "B_w_down": _B_in["w_down"],
        "gate_w": _w((lambda *s: _rng.normal(s) * 0.05)(448) * 16.0),
    }

def reference(A_x, A_Lambda_re, A_Lambda_im, A_B_re, A_B_im, A_C_re, A_C_im, A_log_dt, A_Dskip, B_x, B_w_gate, B_w_up, B_w_down, gate_w):
    def _A_ref(x, Lambda_re, Lambda_im, B_re, B_im, C_re, C_im, log_dt, Dskip):
        Bsz, L, H = x.shape
        Lam = Lambda_re + 1j * Lambda_im
        Bmat = B_re + 1j * B_im
        Cmat = C_re + 1j * C_im
        dt = jnp.exp(log_dt)
        Lam_bar = jnp.exp(dt * Lam)
        B_bar = ((Lam_bar - 1.0) / Lam)[:, None] * Bmat
        Bu = jnp.einsum("bld,pd->blp", x + 0j, B_bar)
        h = jnp.zeros_like(Bu[:, 0, :])
        hs = []
        for t in range(L):
            h = Lam_bar[None, :] * h + Bu[:, t, :]
            hs.append(h)
        hseq = jnp.stack(hs, 1)
        y = 2.0 * jnp.einsum("blp,dp->bld", hseq, Cmat).real + x * Dskip[None, None, :]
        return y

    def _B_ref(x, w_gate, w_up, w_down):
        g = jnp.einsum("bsd,df->bsf", x, w_gate)
        u = jnp.einsum("bsd,df->bsf", x, w_up)
        h = _gelu(g) * u
        return jnp.einsum("bsf,fd->bsd", h, w_down)

    x = A_x
    g = _sigmoid((x * gate_w).sum(-1, keepdims=True))
    a = _A_ref(x, A_Lambda_re, A_Lambda_im, A_B_re, A_B_im, A_C_re, A_C_im, A_log_dt, A_Dskip)
    b = _B_ref(x, B_w_gate, B_w_up, B_w_down)
    return g * a + (1 - g) * b
```

```python
import functools

import jax
import jax.numpy as jnp
from jax import lax
import jax.experimental.pallas as pl
import jax.experimental.pallas.tpu as pltpu

_NT = (((1,), (1,)), ((), ()))

T_BLOCK = 512
F_CHUNK = 256
N_SEG = 8
LANES = 128
SEG_PAD = 8


def _gelu_tanh(x):
    c = 0.7978845608028654
    return x * (0.5 * (1.0 + jnp.tanh(c * (x + 0.044715 * (x * x * x)))))


def _cmul(ar, ai, br, bi):
    return ar * br - ai * bi, ar * bi + ai * br


def _kernel(xt_ref, lre_ref, lim_ref, logdt_ref, dskip_ref, gw_ref,
            bre_hbm, bim_hbm, cre_hbm, cim_hbm, wg_hbm, wu_hbm, wdt_hbm,
            o_ref,
            sr_ref, si_ref, car_ref, cai_ref, dcol_ref,
            bre_v, bim_v, cre_v, cim_v, wg_v, wu_v, wdt_v, sems):
    d, tb = xt_ref.shape
    seg = tb // N_SEG
    pitch = seg + SEG_PAD
    p = lre_ref.shape[0]
    df = wg_hbm.shape[1]
    nch = df // F_CHUNK
    f32 = jnp.float32
    bf16 = jnp.bfloat16
    groups = [(o, min(LANES, p - o)) for o in range(0, p, LANES)]
    ng = len(groups)

    def cp_full(k, src, dst):
        return pltpu.make_async_copy(src, dst, sems.at[k])

    def cp_chunk(k, src, dst, j):
        sl = pl.ds(j * F_CHUNK, F_CHUNK)
        return pltpu.make_async_copy(src.at[:, sl], dst.at[:, sl], sems.at[k])

    def all_copies():
        cps = [cp_full(0, bre_hbm, bre_v), cp_full(1, bim_hbm, bim_v)]
        for j in range(nch):
            cps.append(cp_chunk(4 + 3 * j, wg_hbm, wg_v, j))
            cps.append(cp_chunk(5 + 3 * j, wu_hbm, wu_v, j))
            cps.append(cp_chunk(6 + 3 * j, wdt_hbm, wdt_v, j))
        cps += [cp_full(2, cre_hbm, cre_v), cp_full(3, cim_hbm, cim_v)]
        return cps

    def body(first):
        def wait(make_copy, *args):
            if first:
                make_copy(*args).wait()

        xt = xt_ref[...]
        x = xt.T

        lam_re = lre_ref[...].astype(f32).reshape(1, p)
        lam_im = lim_ref[...].astype(f32).reshape(1, p)
        dt = jnp.exp(logdt_ref[...].astype(f32).reshape(1, p))
        dt = dt.astype(bf16).astype(f32)
        e = jnp.exp(dt * lam_re)
        ang = dt * lam_im
        lbr = e * jnp.cos(ang)
        lbi = e * jnp.sin(ang)
        den = lam_re * lam_re + lam_im * lam_im
        nr = lbr - 1.0
        fr = (nr * lam_re + lbi * lam_im) / den
        fi = (lbi * lam_re - nr * lam_im) / den
        mr, mi = lbr, lbi
        k = 1
        while k < seg:
            mr, mi = mr * mr - mi * mi, 2.0 * mr * mi
            k *= 2
        assert k == seg

        def g8(v, g):
            o, w = groups[g]
            return jnp.broadcast_to(v[:, o:o + w], (N_SEG, w))

        lbr8 = [g8(lbr, g) for g in range(ng)]
        lbi8 = [g8(lbi, g) for g in range(ng)]
        fr8 = [g8(fr, g) for g in range(ng)]
        fi8 = [g8(fi, g) for g in range(ng)]

        wait(cp_full, 0, bre_hbm, bre_v)
        wait(cp_full, 1, bim_hbm, bim_v)
        for g, (o, w) in enumerate(groups):
            for ref, b_v in ((sr_ref, bre_v), (si_ref, bim_v)):
                bu = lax.dot_general(x, b_v[o:o + w, :], _NT,
                                     preferred_element_type=f32)
                for c in range(N_SEG):
                    ref[g, c * pitch:c * pitch + seg, :w] = (
                        bu[c * seg:(c + 1) * seg])

        def ld(ref, g, i):
            return ref[g, pl.ds(i, N_SEG, stride=pitch), :groups[g][1]]

        lr = [jnp.zeros((N_SEG, w), f32) for _, w in groups]
        li = [jnp.zeros((N_SEG, w), f32) for _, w in groups]
        for i in range(seg):
            for g in range(ng):
                tr, ti = _cmul(lbr8[g], lbi8[g], lr[g], li[g])
                lr[g] = tr + ld(sr_ref, g, i)
                li[g] = ti + ld(si_ref, g, i)

        hr, hi = [], []
        for g, (o, w) in enumerate(groups):
            row = lax.broadcasted_iota(jnp.int32, (N_SEG, w), 0)
            first_row = row == 0
            kr, ki = mr[:, o:o + w], mi[:, o:o + w]
            pr = pltpu.roll(car_ref[g, :, :w], 1, 0)
            pi = pltpu.roll(cai_ref[g, :, :w], 1, 0)
            tr, ti = _cmul(kr, ki, pr, pi)
            ar = lr[g] + jnp.where(first_row, tr, 0.0)
            ai = li[g] + jnp.where(first_row, ti, 0.0)
            for s in (1, 2, 4):
                rr = pltpu.roll(ar, s, 0)
                ri = pltpu.roll(ai, s, 0)
                tr, ti = _cmul(kr, ki, rr, ri)
                keep = row >= s
                ar = ar + jnp.where(keep, tr, 0.0)
                ai = ai + jnp.where(keep, ti, 0.0)
                kr, ki = kr * kr - ki * ki, 2.0 * kr * ki
            hr.append(jnp.where(first_row, pr, pltpu.roll(ar, 1, 0)))
            hi.append(jnp.where(first_row, pi, pltpu.roll(ai, 1, 0)))
            car_ref[g, :, :w] = ar
            cai_ref[g, :, :w] = ai

        for i in range(seg):
            for g, (o, w) in enumerate(groups):
                tr, ti = _cmul(lbr8[g], lbi8[g], hr[g], hi[g])
                hr[g] = tr + ld(sr_ref, g, i)
                hi[g] = ti + ld(si_ref, g, i)
                qr, qi = _cmul(fr8[g], fi8[g], hr[g], hi[g])
                sr_ref[g, pl.ds(i, N_SEG, stride=pitch), :w] = qr
                si_ref[g, pl.ds(i, N_SEG, stride=pitch), :w] = qi

        bt = None
        for j in range(nch):
            sl = slice(j * F_CHUNK, (j + 1) * F_CHUNK)
            wait(cp_chunk, 4 + 3 * j, wg_hbm, wg_v, j)
            g_ = jnp.dot(x, wg_v[:, sl], preferred_element_type=f32)
            wait(cp_chunk, 5 + 3 * j, wu_hbm, wu_v, j)
            u_ = jnp.dot(x, wu_v[:, sl], preferred_element_type=f32)
            h = (_gelu_tanh(g_) * u_).astype(bf16)
            wait(cp_chunk, 6 + 3 * j, wdt_hbm, wdt_v, j)
            t = lax.dot_general(wdt_v[:, sl], h, _NT,
                                preferred_element_type=f32)
            bt = t if bt is None else bt + t

        def seg_rows(ref, g, w):
            return jnp.concatenate(
                [ref[g, c * pitch:c * pitch + seg, :w] for c in range(N_SEG)],
                axis=0).astype(bf16)

        wait(cp_full, 2, cre_hbm, cre_v)
        wait(cp_full, 3, cim_hbm, cim_v)
        at = None
        for g, (o, w) in enumerate(groups):
            t = lax.dot_general(cre_v[:, o:o + w], seg_rows(sr_ref, g, w),
                                _NT, preferred_element_type=f32)
            t = t - lax.dot_general(cim_v[:, o:o + w],
                                    seg_rows(si_ref, g, w), _NT,
                                    preferred_element_type=f32)
            at = t if at is None else at + t
        at = 2.0 * at + xt.astype(f32) * dcol_ref[...]

        z = jnp.dot(gw_ref[...].reshape(1, d), xt,
                    preferred_element_type=f32)
        z = z.astype(bf16).astype(f32)
        gate = (1.0 / (1.0 + jnp.exp(-z))).astype(bf16)
        omg = (1.0 - gate).astype(f32)
        o_ref[...] = gate.astype(f32) * at + omg * bt

    step = pl.program_id(0)

    @pl.when(step == 0)
    def _():
        for c in all_copies():
            c.start()
        car_ref[...] = jnp.zeros(car_ref.shape, f32)
        cai_ref[...] = jnp.zeros(cai_ref.shape, f32)
        dsk = dskip_ref[...].astype(f32).reshape(1, d)
        dcol_ref[...] = jnp.broadcast_to(dsk, (tb, d)).T
        body(True)

    @pl.when(step > 0)
    def _():
        body(False)


@jax.jit
def pallas_gated_mix__ssm_conv_s5__glu_gated_geglu__prompt_kernel(
    A_x: jax.Array,
    A_Lambda_re: jax.Array,
    A_Lambda_im: jax.Array,
    A_B_re: jax.Array,
    A_B_im: jax.Array,
    A_C_re: jax.Array,
    A_C_im: jax.Array,
    A_log_dt: jax.Array,
    A_Dskip: jax.Array,
    B_x: jax.Array,
    B_w_gate: jax.Array,
    B_w_up: jax.Array,
    B_w_down: jax.Array,
    gate_w: jax.Array,
):
    del B_x
    bsz, seq, d = A_x.shape
    assert bsz == 1
    p = A_Lambda_re.shape[0]
    df = B_w_gate.shape[1]
    xt = A_x.reshape(seq, d).T
    wdt = B_w_down.T

    tb = T_BLOCK
    seg = tb // N_SEG
    grid = (seq // tb,)
    hbm = pl.BlockSpec(memory_space=pl.ANY)
    vec = lambda n: pl.BlockSpec((n,), lambda i: (0,))
    ng = pl.cdiv(p, LANES)
    ncopies = 4 + 3 * (df // F_CHUNK)
    bf = jnp.bfloat16

    out_t = pl.pallas_call(
        _kernel,
        grid=grid,
        in_specs=[
            pl.BlockSpec((d, tb), lambda i: (0, i)),
            vec(p), vec(p), vec(p), vec(d), vec(d),
            hbm, hbm, hbm, hbm, hbm, hbm, hbm,
        ],
        out_specs=pl.BlockSpec((d, tb), lambda i: (0, i)),
        out_shape=jax.ShapeDtypeStruct((d, seq), jnp.float32),
        scratch_shapes=[
            pltpu.VMEM((ng, N_SEG * (seg + SEG_PAD), LANES), jnp.float32),
            pltpu.VMEM((ng, N_SEG * (seg + SEG_PAD), LANES), jnp.float32),
            pltpu.VMEM((ng, N_SEG, LANES), jnp.float32),
            pltpu.VMEM((ng, N_SEG, LANES), jnp.float32),
            pltpu.VMEM((d, tb), jnp.float32),
            pltpu.VMEM((p, d), bf), pltpu.VMEM((p, d), bf),
            pltpu.VMEM((d, p), bf), pltpu.VMEM((d, p), bf),
            pltpu.VMEM((d, df), bf), pltpu.VMEM((d, df), bf),
            pltpu.VMEM((d, df), bf),
            pltpu.SemaphoreType.DMA((ncopies,)),
        ],
        compiler_params=pltpu.CompilerParams(
            dimension_semantics=("arbitrary",),
            vmem_limit_bytes=100 * 1024 * 1024,
        ),
    )(xt, A_Lambda_re, A_Lambda_im, A_log_dt, A_Dskip,
      gate_w, A_B_re, A_B_im, A_C_re, A_C_im, B_w_gate, B_w_up, wdt)
    return out_t.T.reshape(bsz, seq, d)
```

```python
import functools

import jax
import jax.numpy as jnp
from jax import lax
import jax.experimental.pallas as pl
import jax.experimental.pallas.tpu as pltpu

_NT = (((1,), (1,)), ((), ()))

T_BLOCK = 512
F_CHUNKS = (1792,)
N_SEG = 8
LANES = 128
OUT_SLAB = 128
SEG_PAD = 8


def _gelu_tanh(x):
    c = 0.7978845608028654
    return x * (0.5 * (1.0 + jnp.tanh(c * (x + 0.044715 * (x * x * x)))))


def _cmul(ar, ai, br, bi):
    return ar * br - ai * bi, ar * bi + ai * br


def _kernel(nblk, xt_ref, lre_ref, lim_ref, logdt_ref, dskip_ref, gw_ref,
            bre_hbm, bim_hbm, cre_hbm, cim_hbm, wg_hbm, wu_hbm, wdt_hbm,
            o_hbm,
            sr_ref, si_ref, car_ref, cai_ref, dcol_ref,
            bre_v, bim_v, cre_v, cim_v, wg_v, wu_v, wdt_v,
            bcomb_v, ccomb_v, obuf, sems, osems):
    d, tb = xt_ref.shape
    seg = tb // N_SEG
    pitch = seg + SEG_PAD
    p = lre_ref.shape[0]
    df = wg_hbm.shape[1]
    assert sum(F_CHUNKS) == df
    assert OUT_SLAB % seg == 0 and tb % OUT_SLAB == 0
    nch = len(F_CHUNKS)
    f_off = [sum(F_CHUNKS[:j]) for j in range(nch)]
    f32 = jnp.float32
    bf16 = jnp.bfloat16
    groups = [(o, min(LANES, p - o)) for o in range(0, p, LANES)]
    ng = len(groups)
    rem = p % LANES
    merged = 0 < rem <= LANES // 2
    nfull = ng - 1 if merged else ng
    o_rem = p - rem

    stages = [[('bre', bre_hbm, bre_v, None), ('bim', bim_hbm, bim_v, None)]]
    for j in range(nch):
        csl = (f_off[j], F_CHUNKS[j])
        stages.append([('wg', wg_hbm, wg_v, csl)])
        stages.append([('wu', wu_hbm, wu_v, csl)])
        stages.append([('wdt', wdt_hbm, wdt_v, csl)])
    stages[-1] += [('cre', cre_hbm, cre_v, None), ('cim', cim_hbm, cim_v, None)]
    stages.append([])
    sem_ids = {}
    for st in stages:
        for c in st:
            sem_ids[(c[0], c[3])] = len(sem_ids)
    assert len(sem_ids) == sems.shape[0]

    def make_copy(c):
        nm, src, dst, csl = c
        if csl is not None:
            src = src.at[:, pl.ds(*csl)]
            dst = dst.at[:, pl.ds(*csl)]
        return pltpu.make_async_copy(src, dst, sems.at[sem_ids[(nm, csl)]])

    nslab = tb // OUT_SLAB

    def out_copy(stp, q):
        par = stp % 2
        tsl_ = pl.ds(q * OUT_SLAB, OUT_SLAB)
        return pltpu.make_async_copy(
            obuf.at[par, :, tsl_],
            o_hbm.at[:, pl.ds(stp * tb + q * OUT_SLAB, OUT_SLAB)],
            osems.at[par, q])

    def stage_a(first):
        def use(k):
            if first:
                for c in stages[k]:
                    make_copy(c).wait()
                for c in stages[k + 1]:
                    make_copy(c).start()

        xt = xt_ref[...]
        x = xt.T

        lam_re = lre_ref[...].astype(f32).reshape(1, p)
        lam_im = lim_ref[...].astype(f32).reshape(1, p)
        dt = jnp.exp(logdt_ref[...].astype(f32).reshape(1, p))
        dt = dt.astype(bf16).astype(f32)
        e = jnp.exp(dt * lam_re)
        ang = dt * lam_im
        lbr = e * jnp.cos(ang)
        lbi = e * jnp.sin(ang)
        den = lam_re * lam_re + lam_im * lam_im
        nr = lbr - 1.0
        fr = (nr * lam_re + lbi * lam_im) / den
        fi = (lbi * lam_re - nr * lam_im) / den
        mr, mi = lbr, lbi
        k = 1
        while k < seg:
            mr, mi = mr * mr - mi * mi, 2.0 * mr * mi
            k *= 2
        assert k == seg

        def g8(v, g):
            o, w = groups[g]
            return jnp.broadcast_to(v[:, o:o + w], (N_SEG, w))

        lbr8 = [g8(lbr, g) for g in range(ng)]
        lbi8 = [g8(lbi, g) for g in range(ng)]
        fr8 = [g8(fr, g) for g in range(ng)]
        fi8 = [g8(fi, g) for g in range(ng)]

        use(0)

        def put_segments(ref, g, val):
            for c in range(N_SEG):
                ref[g, c * pitch:c * pitch + seg, :val.shape[1]] = (
                    val[c * seg:(c + 1) * seg])

        for g, (o, w) in enumerate(groups[:nfull]):
            for ref, b_v in ((sr_ref, bre_v), (si_ref, bim_v)):
                put_segments(ref, g, lax.dot_general(
                    x, b_v[o:o + w, :], _NT, preferred_element_type=f32))
        if merged:
            if first:
                bcomb_v[...] = jnp.zeros(bcomb_v.shape, bf16)
                bcomb_v[0:rem, :] = bre_v[o_rem:p, :]
                bcomb_v[rem:2 * rem, :] = bim_v[o_rem:p, :]
            v = lax.dot_general(x, bcomb_v[...], _NT,
                                preferred_element_type=f32)
            put_segments(sr_ref, ng - 1, v)
            put_segments(si_ref, ng - 1, pltpu.roll(v, LANES - rem, 1))

        def ld(ref, g, i):
            return ref[g, pl.ds(i, N_SEG, stride=pitch), :groups[g][1]]

        lr = [jnp.zeros((N_SEG, w), f32) for _, w in groups]
        li = [jnp.zeros((N_SEG, w), f32) for _, w in groups]
        for i in range(seg):
            for g in range(ng):
                tr, ti = _cmul(lbr8[g], lbi8[g], lr[g], li[g])
                lr[g] = tr + ld(sr_ref, g, i)
                li[g] = ti + ld(si_ref, g, i)

        hr, hi = [], []
        for g, (o, w) in enumerate(groups):
            row = lax.broadcasted_iota(jnp.int32, (N_SEG, w), 0)
            first_row = row == 0
            kr, ki = mr[:, o:o + w], mi[:, o:o + w]
            pr = pltpu.roll(car_ref[g, :, :w], 1, 0)
            pi = pltpu.roll(cai_ref[g, :, :w], 1, 0)
            tr, ti = _cmul(kr, ki, pr, pi)
            ar = lr[g] + jnp.where(first_row, tr, 0.0)
            ai = li[g] + jnp.where(first_row, ti, 0.0)
            for s in (1, 2, 4):
                rr = pltpu.roll(ar, s, 0)
                ri = pltpu.roll(ai, s, 0)
                tr, ti = _cmul(kr, ki, rr, ri)
                keep = row >= s
                ar = ar + jnp.where(keep, tr, 0.0)
                ai = ai + jnp.where(keep, ti, 0.0)
                kr, ki = kr * kr - ki * ki, 2.0 * kr * ki
            hr.append(jnp.where(first_row, pr, pltpu.roll(ar, 1, 0)))
            hi.append(jnp.where(first_row, pi, pltpu.roll(ai, 1, 0)))
            car_ref[g, :, :w] = ar
            cai_ref[g, :, :w] = ai

        for i in range(seg):
            for g, (o, w) in enumerate(groups):
                tr, ti = _cmul(lbr8[g], lbi8[g], hr[g], hi[g])
                hr[g] = tr + ld(sr_ref, g, i)
                hi[g] = ti + ld(si_ref, g, i)
                qr, qi = _cmul(fr8[g], fi8[g], hr[g], hi[g])
                sr_ref[g, pl.ds(i, N_SEG, stride=pitch), :w] = qr
                si_ref[g, pl.ds(i, N_SEG, stride=pitch), :w] = qi

        bt = None
        for j in range(nch):
            sl = slice(f_off[j], f_off[j] + F_CHUNKS[j])
            use(1 + 3 * j)
            g_ = jnp.dot(x, wg_v[:, sl], preferred_element_type=f32)
            use(2 + 3 * j)
            u_ = jnp.dot(x, wu_v[:, sl], preferred_element_type=f32)
            h = (_gelu_tanh(g_) * u_).astype(bf16)
            use(3 + 3 * j)
            t = lax.dot_general(wdt_v[:, sl], h, _NT,
                                preferred_element_type=f32)
            bt = t if bt is None else bt + t
        if merged and first:
            ccomb_v[...] = jnp.zeros(ccomb_v.shape, bf16)
            ccomb_v[:, 0:rem] = cre_v[:, o_rem:p]
            ccomb_v[:, rem:2 * rem] = -cim_v[:, o_rem:p]

        z = jnp.dot(gw_ref[...].reshape(1, d), xt,
                    preferred_element_type=f32)
        z = z.astype(bf16).astype(f32)
        gate = (1.0 / (1.0 + jnp.exp(-z))).astype(bf16)
        omg = (1.0 - gate).astype(f32)
        gate = gate.astype(f32)
        stage_b(bt, gate, omg, xt)

    def stage_b(bt, gate, omg, xt):
        for q in range(tb // OUT_SLAB):
            t0 = q * OUT_SLAB
            tsl = slice(t0, t0 + OUT_SLAB)
            segs = range(t0 // seg, (t0 + OUT_SLAB) // seg)

            def seg_rows(ref, g, w, dtype=bf16):
                return jnp.concatenate(
                    [ref[g, c * pitch:c * pitch + seg, :w] for c in segs],
                    axis=0).astype(dtype)

            at = None
            for g, (o, w) in enumerate(groups[:nfull]):
                t = lax.dot_general(cre_v[:, o:o + w], seg_rows(sr_ref, g, w),
                                    _NT, preferred_element_type=f32)
                t = t - lax.dot_general(cim_v[:, o:o + w],
                                        seg_rows(si_ref, g, w), _NT,
                                        preferred_element_type=f32)
                at = t if at is None else at + t
            if merged:
                lo = seg_rows(sr_ref, ng - 1, LANES, f32)
                hi_ = pltpu.roll(seg_rows(si_ref, ng - 1, LANES, f32), rem, 1)
                lane = lax.broadcasted_iota(jnp.int32, lo.shape, 1)
                hc = jnp.where(lane < rem, lo, hi_).astype(bf16)
                t = lax.dot_general(ccomb_v[...], hc, _NT,
                                    preferred_element_type=f32)
                at = t if at is None else at + t
            at = 2.0 * at + xt[:, tsl].astype(f32) * dcol_ref[:, tsl]
            obuf[step % 2, :, tsl] = (gate[:, tsl] * at
                                      + omg[:, tsl] * bt[:, tsl])
            out_copy(step, q).start()

    step = pl.program_id(0)
    nsteps = pl.num_programs(0)

    @pl.when(step >= 2)
    def _():
        for q in range(nslab):
            out_copy(step - 2, q).wait()

    @pl.when(step == 0)
    def _():
        for c in stages[0]:
            make_copy(c).start()
        car_ref[...] = jnp.zeros(car_ref.shape, f32)
        cai_ref[...] = jnp.zeros(cai_ref.shape, f32)
        dsk = dskip_ref[...].astype(f32).reshape(1, d)
        dcol_ref[...] = jnp.broadcast_to(dsk, (tb, d)).T
        stage_a(True)

    @pl.when(step > 0)
    def _():
        stage_a(False)

    @pl.when(step == nsteps - 1)
    def _():
        if nblk >= 2:
            for q in range(nslab):
                out_copy(step - 1, q).wait()
        for q in range(nslab):
            out_copy(step, q).wait()


@jax.jit
def pallas_gated_mix__ssm_conv_s5__glu_gated_geglu__prompt_kernel(
    A_x: jax.Array,
    A_Lambda_re: jax.Array,
    A_Lambda_im: jax.Array,
    A_B_re: jax.Array,
    A_B_im: jax.Array,
    A_C_re: jax.Array,
    A_C_im: jax.Array,
    A_log_dt: jax.Array,
    A_Dskip: jax.Array,
    B_x: jax.Array,
    B_w_gate: jax.Array,
    B_w_up: jax.Array,
    B_w_down: jax.Array,
    gate_w: jax.Array,
):
    del B_x
    bsz, seq, d = A_x.shape
    assert bsz == 1
    p = A_Lambda_re.shape[0]
    df = B_w_gate.shape[1]
    xt = A_x.reshape(seq, d).T
    wdt = B_w_down.T

    tb = T_BLOCK
    seg = tb // N_SEG
    nblk = seq // tb
    hbm = pl.BlockSpec(memory_space=pl.ANY)
    vec = lambda n: pl.BlockSpec((n,), lambda i: (0,))
    ng = pl.cdiv(p, LANES)
    ncopies = 4 + 3 * len(F_CHUNKS)
    bf = jnp.bfloat16
    srows = N_SEG * (seg + SEG_PAD)

    out_t = pl.pallas_call(
        functools.partial(_kernel, nblk),
        grid=(nblk,),
        in_specs=[
            pl.BlockSpec((d, tb), lambda i: (0, i)),
            vec(p), vec(p), vec(p), vec(d), vec(d),
            hbm, hbm, hbm, hbm, hbm, hbm, hbm,
        ],
        out_specs=hbm,
        out_shape=jax.ShapeDtypeStruct((d, seq), jnp.float32),
        scratch_shapes=[
            pltpu.VMEM((ng, srows, LANES), jnp.float32),
            pltpu.VMEM((ng, srows, LANES), jnp.float32),
            pltpu.VMEM((ng, N_SEG, LANES), jnp.float32),
            pltpu.VMEM((ng, N_SEG, LANES), jnp.float32),
            pltpu.VMEM((d, tb), jnp.float32),
            pltpu.VMEM((p, d), bf), pltpu.VMEM((p, d), bf),
            pltpu.VMEM((d, p), bf), pltpu.VMEM((d, p), bf),
            pltpu.VMEM((d, df), bf), pltpu.VMEM((d, df), bf),
            pltpu.VMEM((d, df), bf),
            pltpu.VMEM((LANES, d), bf), pltpu.VMEM((d, LANES), bf),
            pltpu.VMEM((2, d, tb), jnp.float32),
            pltpu.SemaphoreType.DMA((ncopies,)),
            pltpu.SemaphoreType.DMA((2, tb // OUT_SLAB)),
        ],
        compiler_params=pltpu.CompilerParams(
            dimension_semantics=("arbitrary",),
            vmem_limit_bytes=100 * 1024 * 1024,
        ),
    )(xt, A_Lambda_re, A_Lambda_im, A_log_dt, A_Dskip,
      gate_w, A_B_re, A_B_im, A_C_re, A_C_im, B_w_gate, B_w_up, wdt)
    return out_t.T.reshape(bsz, seq, d)
```

```python
import functools

import jax
import jax.numpy as jnp
from jax import lax
import jax.experimental.pallas as pl
import jax.experimental.pallas.tpu as pltpu

_NT = (((1,), (1,)), ((), ()))

T_BLOCK = 512
F_CHUNKS = (1792,)
N_SEG = 8
LANES = 128
OUT_SLAB = 128
SEG_PAD = 8


def _gelu_tanh(x):
    c = 0.7978845608028654
    return x * (0.5 * (1.0 + jnp.tanh(c * (x + 0.044715 * (x * x * x)))))


def _cmul(ar, ai, br, bi):
    return ar * br - ai * bi, ar * bi + ai * br


def _kernel(nblk, xt_ref, lre_ref, lim_ref, logdt_ref, dskip_ref, gw_ref,
            bre_hbm, bim_hbm, cre_hbm, cim_hbm, wg_hbm, wu_hbm, wdt_hbm, xt_hbm,
            o_hbm,
            sr_ref, si_ref, car_ref, cai_ref, dcol_ref,
            bre_v, bim_v, cre_v, cim_v, wg_v, wu_v, wdt_v,
            bcomb_v, ccomb_v, obuf, xraw, xbuf, sems, osems, xsems):
    d, tb = xt_ref.shape
    seg = tb // N_SEG
    pitch = seg + SEG_PAD
    p = lre_ref.shape[0]
    df = wg_hbm.shape[1]
    assert sum(F_CHUNKS) == df
    assert OUT_SLAB % seg == 0 and tb % OUT_SLAB == 0
    nch = len(F_CHUNKS)
    f_off = [sum(F_CHUNKS[:j]) for j in range(nch)]
    f32 = jnp.float32
    bf16 = jnp.bfloat16
    groups = [(o, min(LANES, p - o)) for o in range(0, p, LANES)]
    ng = len(groups)
    rem = p % LANES
    merged = 0 < rem <= LANES // 2
    nfull = ng - 1 if merged else ng
    o_rem = p - rem

    stages = [[('bre', bre_hbm, bre_v, None), ('bim', bim_hbm, bim_v, None)]]
    for j in range(nch):
        csl = (f_off[j], F_CHUNKS[j])
        stages.append([('wg', wg_hbm, wg_v, csl)])
        stages.append([('wu', wu_hbm, wu_v, csl)])
        stages.append([('wdt', wdt_hbm, wdt_v, csl)])
    stages[-1] += [('cre', cre_hbm, cre_v, None), ('cim', cim_hbm, cim_v, None)]
    stages.append([])
    sem_ids = {}
    for st in stages:
        for c in st:
            sem_ids[(c[0], c[3])] = len(sem_ids)
    assert len(sem_ids) == sems.shape[0]

    def make_copy(c):
        nm, src, dst, csl = c
        if csl is not None:
            src = src.at[:, pl.ds(*csl)]
            dst = dst.at[:, pl.ds(*csl)]
        return pltpu.make_async_copy(src, dst, sems.at[sem_ids[(nm, csl)]])

    nslab = tb // OUT_SLAB

    def out_copy(stp, q):
        par = stp % 2
        tsl_ = pl.ds(q * OUT_SLAB, OUT_SLAB)
        return pltpu.make_async_copy(
            obuf.at[par, :, tsl_],
            o_hbm.at[:, pl.ds(stp * tb + q * OUT_SLAB, OUT_SLAB)],
            osems.at[par, q])

    def x_copy(blk):
        return pltpu.make_async_copy(
            xt_hbm.at[:, pl.ds(blk * tb, tb)], xraw.at[blk % 2],
            xsems.at[blk % 2])

    def stage_a(first):
        def use(k):
            if first:
                for c in stages[k]:
                    make_copy(c).wait()
                for c in stages[k + 1]:
                    make_copy(c).start()

        xt = xt_ref[...]
        x = xt.T if first else xbuf[step % 2]
        if not first:
            xbuf[(step + 1) % 2] = xraw[(step + 1) % 2].T

        lam_re = lre_ref[...].astype(f32).reshape(1, p)
        lam_im = lim_ref[...].astype(f32).reshape(1, p)
        dt = jnp.exp(logdt_ref[...].astype(f32).reshape(1, p))
        dt = dt.astype(bf16).astype(f32)
        e = jnp.exp(dt * lam_re)
        ang = dt * lam_im
        lbr = e * jnp.cos(ang)
        lbi = e * jnp.sin(ang)
        den = lam_re * lam_re + lam_im * lam_im
        nr = lbr - 1.0
        fr = (nr * lam_re + lbi * lam_im) / den
        fi = (lbi * lam_re - nr * lam_im) / den
        mr, mi = lbr, lbi
        k = 1
        while k < seg:
            mr, mi = mr * mr - mi * mi, 2.0 * mr * mi
            k *= 2
        assert k == seg

        def g8(v, g):
            o, w = groups[g]
            return jnp.broadcast_to(v[:, o:o + w], (N_SEG, w))

        lbr8 = [g8(lbr, g) for g in range(ng)]
        lbi8 = [g8(lbi, g) for g in range(ng)]
        fr8 = [g8(fr, g) for g in range(ng)]
        fi8 = [g8(fi, g) for g in range(ng)]

        use(0)

        def put_segments(ref, g, val):
            for c in range(N_SEG):
                ref[g, c * pitch:c * pitch + seg, :val.shape[1]] = (
                    val[c * seg:(c + 1) * seg])

        for g, (o, w) in enumerate(groups[:nfull]):
            for ref, b_v in ((sr_ref, bre_v), (si_ref, bim_v)):
                put_segments(ref, g, lax.dot_general(
                    x, b_v[o:o + w, :], _NT, preferred_element_type=f32))
        if merged:
            if first:
                bcomb_v[...] = jnp.zeros(bcomb_v.shape, bf16)
                bcomb_v[0:rem, :] = bre_v[o_rem:p, :]
                bcomb_v[rem:2 * rem, :] = bim_v[o_rem:p, :]
            v = lax.dot_general(x, bcomb_v[...], _NT,
                                preferred_element_type=f32)
            put_segments(sr_ref, ng - 1, v)
            put_segments(si_ref, ng - 1, pltpu.roll(v, LANES - rem, 1))

        def ld(ref, g, i):
            return ref[g, pl.ds(i, N_SEG, stride=pitch), :groups[g][1]]

        lr = [jnp.zeros((N_SEG, w), f32) for _, w in groups]
        li = [jnp.zeros((N_SEG, w), f32) for _, w in groups]
        for i in range(seg):
            for g in range(ng):
                tr, ti = _cmul(lbr8[g], lbi8[g], lr[g], li[g])
                lr[g] = tr + ld(sr_ref, g, i)
                li[g] = ti + ld(si_ref, g, i)

        hr, hi = [], []
        for g, (o, w) in enumerate(groups):
            row = lax.broadcasted_iota(jnp.int32, (N_SEG, w), 0)
            first_row = row == 0
            kr, ki = mr[:, o:o + w], mi[:, o:o + w]
            pr = pltpu.roll(car_ref[g, :, :w], 1, 0)
            pi = pltpu.roll(cai_ref[g, :, :w], 1, 0)
            tr, ti = _cmul(kr, ki, pr, pi)
            ar = lr[g] + jnp.where(first_row, tr, 0.0)
            ai = li[g] + jnp.where(first_row, ti, 0.0)
            for s in (1, 2, 4):
                rr = pltpu.roll(ar, s, 0)
                ri = pltpu.roll(ai, s, 0)
                tr, ti = _cmul(kr, ki, rr, ri)
                keep = row >= s
                ar = ar + jnp.where(keep, tr, 0.0)
                ai = ai + jnp.where(keep, ti, 0.0)
                kr, ki = kr * kr - ki * ki, 2.0 * kr * ki
            hr.append(jnp.where(first_row, pr, pltpu.roll(ar, 1, 0)))
            hi.append(jnp.where(first_row, pi, pltpu.roll(ai, 1, 0)))
            car_ref[g, :, :w] = ar
            cai_ref[g, :, :w] = ai

        for i in range(seg):
            for g, (o, w) in enumerate(groups):
                tr, ti = _cmul(lbr8[g], lbi8[g], hr[g], hi[g])
                hr[g] = tr + ld(sr_ref, g, i)
                hi[g] = ti + ld(si_ref, g, i)
                qr, qi = _cmul(fr8[g], fi8[g], hr[g], hi[g])
                sr_ref[g, pl.ds(i, N_SEG, stride=pitch), :w] = qr
                si_ref[g, pl.ds(i, N_SEG, stride=pitch), :w] = qi

        bt = None
        for j in range(nch):
            sl = slice(f_off[j], f_off[j] + F_CHUNKS[j])
            use(1 + 3 * j)
            g_ = jnp.dot(x, wg_v[:, sl], preferred_element_type=f32)
            use(2 + 3 * j)
            u_ = jnp.dot(x, wu_v[:, sl], preferred_element_type=f32)
            h = (_gelu_tanh(g_) * u_).astype(bf16)
            use(3 + 3 * j)
            t = lax.dot_general(wdt_v[:, sl], h, _NT,
                                preferred_element_type=f32)
            bt = t if bt is None else bt + t
        if first:
            for blk in range(1, min(nblk, 3)):
                x_copy(blk).start()
            if nblk > 1:
                x_copy(1).wait()
                xbuf[1] = xraw[1].T
        if merged and first:
            ccomb_v[...] = jnp.zeros(ccomb_v.shape, bf16)
            ccomb_v[:, 0:rem] = cre_v[:, o_rem:p]
            ccomb_v[:, rem:2 * rem] = -cim_v[:, o_rem:p]

        z = jnp.dot(gw_ref[...].reshape(1, d), xt,
                    preferred_element_type=f32)
        z = z.astype(bf16).astype(f32)
        gate = (1.0 / (1.0 + jnp.exp(-z))).astype(bf16)
        omg = (1.0 - gate).astype(f32)
        gate = gate.astype(f32)
        stage_b(bt, gate, omg, xt)

    def stage_b(bt, gate, omg, xt):
        for q in range(tb // OUT_SLAB):
            t0 = q * OUT_SLAB
            tsl = slice(t0, t0 + OUT_SLAB)
            segs = range(t0 // seg, (t0 + OUT_SLAB) // seg)

            def seg_rows(ref, g, w, dtype=bf16):
                return jnp.concatenate(
                    [ref[g, c * pitch:c * pitch + seg, :w] for c in segs],
                    axis=0).astype(dtype)

            at = None
            for g, (o, w) in enumerate(groups[:nfull]):
                t = lax.dot_general(cre_v[:, o:o + w], seg_rows(sr_ref, g, w),
                                    _NT, preferred_element_type=f32)
                t = t - lax.dot_general(cim_v[:, o:o + w],
                                        seg_rows(si_ref, g, w), _NT,
                                        preferred_element_type=f32)
                at = t if at is None else at + t
            if merged:
                lo = seg_rows(sr_ref, ng - 1, LANES, f32)
                hi_ = pltpu.roll(seg_rows(si_ref, ng - 1, LANES, f32), rem, 1)
                lane = lax.broadcasted_iota(jnp.int32, lo.shape, 1)
                hc = jnp.where(lane < rem, lo, hi_).astype(bf16)
                t = lax.dot_general(ccomb_v[...], hc, _NT,
                                    preferred_element_type=f32)
                at = t if at is None else at + t
            at = 2.0 * at + xt[:, tsl].astype(f32) * dcol_ref[:, tsl]
            obuf[step % 2, :, tsl] = (gate[:, tsl] * at
                                      + omg[:, tsl] * bt[:, tsl])
            out_copy(step, q).start()

    step = pl.program_id(0)
    nsteps = pl.num_programs(0)

    @pl.when(step >= 2)
    def _():
        for q in range(nslab):
            out_copy(step - 2, q).wait()

    @pl.when(jnp.logical_and(step >= 1, step + 1 < nsteps))
    def _():
        x_copy(step + 1).wait()

    @pl.when(jnp.logical_and(step >= 1, step + 2 < nsteps))
    def _():
        x_copy(step + 2).start()

    @pl.when(step == 0)
    def _():
        for c in stages[0]:
            make_copy(c).start()
        car_ref[...] = jnp.zeros(car_ref.shape, f32)
        cai_ref[...] = jnp.zeros(cai_ref.shape, f32)
        dsk = dskip_ref[...].astype(f32).reshape(1, d)
        dcol_ref[...] = jnp.broadcast_to(dsk, (tb, d)).T
        stage_a(True)

    @pl.when(step > 0)
    def _():
        stage_a(False)

    @pl.when(step == nsteps - 1)
    def _():
        if nblk >= 2:
            for q in range(nslab):
                out_copy(step - 1, q).wait()
        for q in range(nslab):
            out_copy(step, q).wait()


@jax.jit
def pallas_gated_mix__ssm_conv_s5__glu_gated_geglu__prompt_kernel(
    A_x: jax.Array,
    A_Lambda_re: jax.Array,
    A_Lambda_im: jax.Array,
    A_B_re: jax.Array,
    A_B_im: jax.Array,
    A_C_re: jax.Array,
    A_C_im: jax.Array,
    A_log_dt: jax.Array,
    A_Dskip: jax.Array,
    B_x: jax.Array,
    B_w_gate: jax.Array,
    B_w_up: jax.Array,
    B_w_down: jax.Array,
    gate_w: jax.Array,
):
    del B_x
    bsz, seq, d = A_x.shape
    assert bsz == 1
    p = A_Lambda_re.shape[0]
    df = B_w_gate.shape[1]
    xt = A_x.reshape(seq, d).T
    wdt = B_w_down.T

    tb = T_BLOCK
    seg = tb // N_SEG
    nblk = seq // tb
    hbm = pl.BlockSpec(memory_space=pl.ANY)
    vec = lambda n: pl.BlockSpec((n,), lambda i: (0,))
    ng = pl.cdiv(p, LANES)
    ncopies = 4 + 3 * len(F_CHUNKS)
    bf = jnp.bfloat16
    srows = N_SEG * (seg + SEG_PAD)

    out_t = pl.pallas_call(
        functools.partial(_kernel, nblk),
        grid=(nblk,),
        in_specs=[
            pl.BlockSpec((d, tb), lambda i: (0, i)),
            vec(p), vec(p), vec(p), vec(d), vec(d),
            hbm, hbm, hbm, hbm, hbm, hbm, hbm, hbm,
        ],
        out_specs=hbm,
        out_shape=jax.ShapeDtypeStruct((d, seq), jnp.float32),
        scratch_shapes=[
            pltpu.VMEM((ng, srows, LANES), jnp.float32),
            pltpu.VMEM((ng, srows, LANES), jnp.float32),
            pltpu.VMEM((ng, N_SEG, LANES), jnp.float32),
            pltpu.VMEM((ng, N_SEG, LANES), jnp.float32),
            pltpu.VMEM((d, tb), jnp.float32),
            pltpu.VMEM((p, d), bf), pltpu.VMEM((p, d), bf),
            pltpu.VMEM((d, p), bf), pltpu.VMEM((d, p), bf),
            pltpu.VMEM((d, df), bf), pltpu.VMEM((d, df), bf),
            pltpu.VMEM((d, df), bf),
            pltpu.VMEM((LANES, d), bf), pltpu.VMEM((d, LANES), bf),
            pltpu.VMEM((2, d, tb), jnp.float32),
            pltpu.VMEM((2, d, tb), bf),
            pltpu.VMEM((2, tb, d), bf),
            pltpu.SemaphoreType.DMA((ncopies,)),
            pltpu.SemaphoreType.DMA((2, tb // OUT_SLAB)),
            pltpu.SemaphoreType.DMA((2,)),
        ],
        compiler_params=pltpu.CompilerParams(
            dimension_semantics=("arbitrary",),
            vmem_limit_bytes=100 * 1024 * 1024,
        ),
    )(xt, A_Lambda_re, A_Lambda_im, A_log_dt, A_Dskip,
      gate_w, A_B_re, A_B_im, A_C_re, A_C_im, B_w_gate, B_w_up, wdt, xt)
    return out_t.T.reshape(bsz, seq, d)
```

```python
import functools

import jax
import jax.numpy as jnp
from jax import lax
import jax.experimental.pallas as pl
import jax.experimental.pallas.tpu as pltpu

_NT = (((1,), (1,)), ((), ()))

T_BLOCK = 512
F_CHUNKS = (1792,)
N_SEG = 8
LANES = 128
OUT_SLAB = 128
SEG_PAD = 8


def _gelu_tanh(x):
    c = 0.7978845608028654
    return x * (0.5 * (1.0 + jnp.tanh(c * (x + 0.044715 * (x * x * x)))))


def _cmul(ar, ai, br, bi):
    return ar * br - ai * bi, ar * bi + ai * br


def _kernel(nblk, xt_ref, lre_ref, lim_ref, logdt_ref, dskip_ref, gw_ref,
            bre_v, bim_v, cre_hbm, cim_hbm, wg_hbm, wu_hbm, wdt_hbm, xt_hbm,
            o_hbm,
            sr_ref, si_ref, car_ref, cai_ref, dcol_ref,
            cre_v, cim_v, wg_v, wu_v, wdt_v,
            bcomb_v, ccomb_v, obuf, xraw, xbuf, sems, osems, xsems):
    d, tb = xt_ref.shape
    seg = tb // N_SEG
    pitch = seg + SEG_PAD
    p = lre_ref.shape[0]
    df = wg_hbm.shape[1]
    assert sum(F_CHUNKS) == df
    assert OUT_SLAB % seg == 0 and tb % OUT_SLAB == 0
    nch = len(F_CHUNKS)
    f_off = [sum(F_CHUNKS[:j]) for j in range(nch)]
    f32 = jnp.float32
    bf16 = jnp.bfloat16
    groups = [(o, min(LANES, p - o)) for o in range(0, p, LANES)]
    ng = len(groups)
    rem = p % LANES
    merged = 0 < rem <= LANES // 2
    nfull = ng - 1 if merged else ng
    o_rem = p - rem

    stages = [[]]
    for j in range(nch):
        csl = (f_off[j], F_CHUNKS[j])
        stages.append([('wg', wg_hbm, wg_v, csl)])
        stages.append([('wu', wu_hbm, wu_v, csl)])
        stages.append([('wdt', wdt_hbm, wdt_v, csl)])
    stages[-1] += [('cre', cre_hbm, cre_v, None), ('cim', cim_hbm, cim_v, None)]
    stages.append([])
    sem_ids = {}
    for st in stages:
        for c in st:
            sem_ids[(c[0], c[3])] = len(sem_ids)
    assert len(sem_ids) == sems.shape[0]

    def make_copy(c):
        nm, src, dst, csl = c
        if csl is not None:
            src = src.at[:, pl.ds(*csl)]
            dst = dst.at[:, pl.ds(*csl)]
        return pltpu.make_async_copy(src, dst, sems.at[sem_ids[(nm, csl)]])

    nslab = tb // OUT_SLAB

    def out_copy(stp, q):
        par = stp % 2
        tsl_ = pl.ds(q * OUT_SLAB, OUT_SLAB)
        return pltpu.make_async_copy(
            obuf.at[par, :, tsl_],
            o_hbm.at[:, pl.ds(stp * tb + q * OUT_SLAB, OUT_SLAB)],
            osems.at[par, q])

    def x_copy(blk):
        return pltpu.make_async_copy(
            xt_hbm.at[:, pl.ds(blk * tb, tb)], xraw.at[blk % 2],
            xsems.at[blk % 2])

    def stage_a(first):
        def use(k):
            if first:
                for c in stages[k]:
                    make_copy(c).wait()
                for c in stages[k + 1]:
                    make_copy(c).start()

        xt = xt_ref[...]
        x = xt.T if first else xbuf[step % 2]
        if not first:
            xbuf[(step + 1) % 2] = xraw[(step + 1) % 2].T

        z = jnp.dot(gw_ref[...].reshape(1, d), xt,
                    preferred_element_type=f32)
        z = z.astype(bf16).astype(f32)
        gate = (1.0 / (1.0 + jnp.exp(-z))).astype(bf16)
        omg = (1.0 - gate).astype(f32)
        gate = gate.astype(f32)

        lam_re = lre_ref[...].astype(f32).reshape(1, p)
        lam_im = lim_ref[...].astype(f32).reshape(1, p)
        dt = jnp.exp(logdt_ref[...].astype(f32).reshape(1, p))
        dt = dt.astype(bf16).astype(f32)
        e = jnp.exp(dt * lam_re)
        ang = dt * lam_im
        lbr = e * jnp.cos(ang)
        lbi = e * jnp.sin(ang)
        den = lam_re * lam_re + lam_im * lam_im
        nr = lbr - 1.0
        fr = (nr * lam_re + lbi * lam_im) / den
        fi = (lbi * lam_re - nr * lam_im) / den
        mr, mi = lbr, lbi
        k = 1
        while k < seg:
            mr, mi = mr * mr - mi * mi, 2.0 * mr * mi
            k *= 2
        assert k == seg

        def g8(v, g):
            o, w = groups[g]
            return jnp.broadcast_to(v[:, o:o + w], (N_SEG, w))

        lbr8 = [g8(lbr, g) for g in range(ng)]
        lbi8 = [g8(lbi, g) for g in range(ng)]
        fr8 = [g8(fr, g) for g in range(ng)]
        fi8 = [g8(fi, g) for g in range(ng)]

        use(0)

        def put_segments(ref, g, val):
            for c in range(N_SEG):
                ref[g, c * pitch:c * pitch + seg, :val.shape[1]] = (
                    val[c * seg:(c + 1) * seg])

        for g, (o, w) in enumerate(groups[:nfull]):
            for ref, b_v in ((sr_ref, bre_v), (si_ref, bim_v)):
                put_segments(ref, g, lax.dot_general(
                    x, b_v[o:o + w, :], _NT, preferred_element_type=f32))
        if merged:
            if first:
                bcomb_v[...] = jnp.zeros(bcomb_v.shape, bf16)
                bcomb_v[0:rem, :] = bre_v[o_rem:p, :]
                bcomb_v[rem:2 * rem, :] = bim_v[o_rem:p, :]
            v = lax.dot_general(x, bcomb_v[...], _NT,
                                preferred_element_type=f32)
            put_segments(sr_ref, ng - 1, v)
            put_segments(si_ref, ng - 1, pltpu.roll(v, LANES - rem, 1))

        def ld(ref, g, i):
            return ref[g, pl.ds(i, N_SEG, stride=pitch), :groups[g][1]]

        lr = [jnp.zeros((N_SEG, w), f32) for _, w in groups]
        li = [jnp.zeros((N_SEG, w), f32) for _, w in groups]
        for i in range(seg):
            for g in range(ng):
                tr, ti = _cmul(lbr8[g], lbi8[g], lr[g], li[g])
                lr[g] = tr + ld(sr_ref, g, i)
                li[g] = ti + ld(si_ref, g, i)

        hr, hi = [], []
        for g, (o, w) in enumerate(groups):
            row = lax.broadcasted_iota(jnp.int32, (N_SEG, w), 0)
            first_row = row == 0
            kr, ki = mr[:, o:o + w], mi[:, o:o + w]
            pr = pltpu.roll(car_ref[g, :, :w], 1, 0)
            pi = pltpu.roll(cai_ref[g, :, :w], 1, 0)
            tr, ti = _cmul(kr, ki, pr, pi)
            ar = lr[g] + jnp.where(first_row, tr, 0.0)
            ai = li[g] + jnp.where(first_row, ti, 0.0)
            for s in (1, 2, 4):
                rr = pltpu.roll(ar, s, 0)
                ri = pltpu.roll(ai, s, 0)
                tr, ti = _cmul(kr, ki, rr, ri)
                keep = row >= s
                ar = ar + jnp.where(keep, tr, 0.0)
                ai = ai + jnp.where(keep, ti, 0.0)
                kr, ki = kr * kr - ki * ki, 2.0 * kr * ki
            hr.append(jnp.where(first_row, pr, pltpu.roll(ar, 1, 0)))
            hi.append(jnp.where(first_row, pi, pltpu.roll(ai, 1, 0)))
            car_ref[g, :, :w] = ar
            cai_ref[g, :, :w] = ai

        for i in range(seg):
            for g, (o, w) in enumerate(groups):
                tr, ti = _cmul(lbr8[g], lbi8[g], hr[g], hi[g])
                hr[g] = tr + ld(sr_ref, g, i)
                hi[g] = ti + ld(si_ref, g, i)
                qr, qi = _cmul(fr8[g], fi8[g], hr[g], hi[g])
                sr_ref[g, pl.ds(i, N_SEG, stride=pitch), :w] = qr
                si_ref[g, pl.ds(i, N_SEG, stride=pitch), :w] = qi

        bt = None
        for j in range(nch):
            sl = slice(f_off[j], f_off[j] + F_CHUNKS[j])
            use(1 + 3 * j)
            g_ = jnp.dot(x, wg_v[:, sl], preferred_element_type=f32)
            use(2 + 3 * j)
            u_ = jnp.dot(x, wu_v[:, sl], preferred_element_type=f32)
            h = (_gelu_tanh(g_) * u_).astype(bf16)
            use(3 + 3 * j)
            t = lax.dot_general(wdt_v[:, sl], h, _NT,
                                preferred_element_type=f32)
            bt = t if bt is None else bt + t
        if first:
            for blk in range(1, min(nblk, 3)):
                x_copy(blk).start()
            if nblk > 1:
                x_copy(1).wait()
                xbuf[1] = xraw[1].T
        if merged and first:
            ccomb_v[...] = jnp.zeros(ccomb_v.shape, bf16)
            ccomb_v[:, 0:rem] = cre_v[:, o_rem:p]
            ccomb_v[:, rem:2 * rem] = -cim_v[:, o_rem:p]

        stage_b(bt, gate, omg, xt)

    def stage_b(bt, gate, omg, xt):
        for q in range(tb // OUT_SLAB):
            t0 = q * OUT_SLAB
            tsl = slice(t0, t0 + OUT_SLAB)
            segs = range(t0 // seg, (t0 + OUT_SLAB) // seg)

            def seg_rows(ref, g, w, dtype=bf16):
                return jnp.concatenate(
                    [ref[g, c * pitch:c * pitch + seg, :w] for c in segs],
                    axis=0).astype(dtype)

            at = None
            for g, (o, w) in enumerate(groups[:nfull]):
                t = lax.dot_general(cre_v[:, o:o + w], seg_rows(sr_ref, g, w),
                                    _NT, preferred_element_type=f32)
                t = t - lax.dot_general(cim_v[:, o:o + w],
                                        seg_rows(si_ref, g, w), _NT,
                                        preferred_element_type=f32)
                at = t if at is None else at + t
            if merged:
                lo = seg_rows(sr_ref, ng - 1, LANES, f32)
                hi_ = pltpu.roll(seg_rows(si_ref, ng - 1, LANES, f32), rem, 1)
                lane = lax.broadcasted_iota(jnp.int32, lo.shape, 1)
                hc = jnp.where(lane < rem, lo, hi_).astype(bf16)
                t = lax.dot_general(ccomb_v[...], hc, _NT,
                                    preferred_element_type=f32)
                at = t if at is None else at + t
            at = 2.0 * at + xt[:, tsl].astype(f32) * dcol_ref[:, tsl]
            obuf[step % 2, :, tsl] = (gate[:, tsl] * at
                                      + omg[:, tsl] * bt[:, tsl])
            out_copy(step, q).start()

    step = pl.program_id(0)
    nsteps = pl.num_programs(0)

    @pl.when(step >= 2)
    def _():
        for q in range(nslab):
            out_copy(step - 2, q).wait()

    @pl.when(jnp.logical_and(step >= 1, step + 1 < nsteps))
    def _():
        x_copy(step + 1).wait()

    @pl.when(jnp.logical_and(step >= 1, step + 2 < nsteps))
    def _():
        x_copy(step + 2).start()

    @pl.when(step == 0)
    def _():
        for c in stages[0]:
            make_copy(c).start()
        car_ref[...] = jnp.zeros(car_ref.shape, f32)
        cai_ref[...] = jnp.zeros(cai_ref.shape, f32)
        dsk = dskip_ref[...].astype(f32).reshape(1, d)
        dcol_ref[...] = jnp.broadcast_to(dsk, (tb, d)).T
        stage_a(True)

    @pl.when(step > 0)
    def _():
        stage_a(False)

    @pl.when(step == nsteps - 1)
    def _():
        if nblk >= 2:
            for q in range(nslab):
                out_copy(step - 1, q).wait()
        for q in range(nslab):
            out_copy(step, q).wait()


@jax.jit
def pallas_gated_mix__ssm_conv_s5__glu_gated_geglu__prompt_kernel(
    A_x: jax.Array,
    A_Lambda_re: jax.Array,
    A_Lambda_im: jax.Array,
    A_B_re: jax.Array,
    A_B_im: jax.Array,
    A_C_re: jax.Array,
    A_C_im: jax.Array,
    A_log_dt: jax.Array,
    A_Dskip: jax.Array,
    B_x: jax.Array,
    B_w_gate: jax.Array,
    B_w_up: jax.Array,
    B_w_down: jax.Array,
    gate_w: jax.Array,
):
    del B_x
    bsz, seq, d = A_x.shape
    assert bsz == 1
    p = A_Lambda_re.shape[0]
    df = B_w_gate.shape[1]
    xt = A_x.reshape(seq, d).T
    wdt = B_w_down.T

    tb = T_BLOCK
    seg = tb // N_SEG
    nblk = seq // tb
    hbm = pl.BlockSpec(memory_space=pl.ANY)
    vec = lambda n: pl.BlockSpec((n,), lambda i: (0,))
    ng = pl.cdiv(p, LANES)
    ncopies = 2 + 3 * len(F_CHUNKS)
    bf = jnp.bfloat16
    srows = N_SEG * (seg + SEG_PAD)

    out_t = pl.pallas_call(
        functools.partial(_kernel, nblk),
        grid=(nblk,),
        in_specs=[
            pl.BlockSpec((d, tb), lambda i: (0, i)),
            vec(p), vec(p), vec(p), vec(d), vec(d),
            pl.BlockSpec((p, d), lambda i: (0, 0)),
            pl.BlockSpec((p, d), lambda i: (0, 0)),
            hbm, hbm, hbm, hbm, hbm, hbm,
        ],
        out_specs=hbm,
        out_shape=jax.ShapeDtypeStruct((d, seq), jnp.float32),
        scratch_shapes=[
            pltpu.VMEM((ng, srows, LANES), jnp.float32),
            pltpu.VMEM((ng, srows, LANES), jnp.float32),
            pltpu.VMEM((ng, N_SEG, LANES), jnp.float32),
            pltpu.VMEM((ng, N_SEG, LANES), jnp.float32),
            pltpu.VMEM((d, tb), jnp.float32),
            pltpu.VMEM((d, p), bf), pltpu.VMEM((d, p), bf),
            pltpu.VMEM((d, df), bf), pltpu.VMEM((d, df), bf),
            pltpu.VMEM((d, df), bf),
            pltpu.VMEM((LANES, d), bf), pltpu.VMEM((d, LANES), bf),
            pltpu.VMEM((2, d, tb), jnp.float32),
            pltpu.VMEM((2, d, tb), bf),
            pltpu.VMEM((2, tb, d), bf),
            pltpu.SemaphoreType.DMA((ncopies,)),
            pltpu.SemaphoreType.DMA((2, tb // OUT_SLAB)),
            pltpu.SemaphoreType.DMA((2,)),
        ],
        compiler_params=pltpu.CompilerParams(
            dimension_semantics=("arbitrary",),
            vmem_limit_bytes=100 * 1024 * 1024,
        ),
    )(xt, A_Lambda_re, A_Lambda_im, A_log_dt, A_Dskip,
      gate_w, A_B_re, A_B_im, A_C_re, A_C_im, B_w_gate, B_w_up, wdt, xt)
    return out_t.T.reshape(bsz, seq, d)
```
